```python
import os as _os
_os.environ.setdefault("JAX_PLATFORMS", "cpu")
import jax
import jax.numpy as jnp

def _softmax(x, axis=-1):
    return jax.nn.softmax(x, axis=axis)
def _gelu(x):
    return jax.nn.gelu(x, approximate=True)
def _silu(x):
    return jax.nn.silu(x)
def _sigmoid(x):
    return jax.nn.sigmoid(x)
def _layernorm(x, axis=-1, eps=1e-5):
    m = jnp.mean(x, axis=axis, keepdims=True)
    v = jnp.var(x, axis=axis, keepdims=True)
    return (x - m) / jnp.sqrt(v + eps)
def _scatter_add(tgt, idx, src, axis=0):
    return tgt.at[idx].add(src)
def _segment_sum(src, seg, n):
    return jax.ops.segment_sum(src, seg, n)
class _Rng:
    def __init__(self, key):
        self._k = key
    def _next(self):
        self._k, sub = jax.random.split(self._k)
        return sub
    def normal(self, shape):
        return jax.random.normal(self._next(), shape, dtype=jnp.bfloat16)
    def randint(self, lo, hi, shape):
        return jax.random.randint(self._next(), shape, lo, hi, dtype=jnp.int32)
    def uniform(self, shape, lo=0.0, hi=1.0):
        return jax.random.uniform(self._next(), shape, jnp.bfloat16, lo, hi)
    def permutation(self, n):
        return jax.random.permutation(self._next(), n)


kernel_name = 'standalone__moe_arch_mod__prompt'

def setup_inputs():
    _rng = _Rng(jax.random.key(int.from_bytes(__import__("os").urandom(4), "little")))
    _w = (lambda a: (lambda t: t.astype(jnp.bfloat16) if jnp.issubdtype(t.dtype, jnp.floating) else t)(jnp.asarray(a)))
    B, S, D, F, C = 1, 2048, 576, 4608, 8
    return {
        "x": _w((lambda *s: _rng.normal(s) * 0.1)(B, S, D)),
        "w_r": _w((lambda *s: _rng.normal(s) * 0.1)(D)),
        "w_gate": _w((lambda *s: _rng.normal(s) * 0.1)(D, F)),
        "w_up": _w((lambda *s: _rng.normal(s) * 0.1)(D, F)),
        "w_down": _w((lambda *s: _rng.normal(s) * 0.1)(F, D)),
    }

def reference(x, w_r, w_gate, w_up, w_down):
    B, S, D = x.shape
    C = 8
    r = x @ w_r
    idx = jnp.argsort(-r, axis=-1)[:, :C]
    idx_e = jnp.repeat(idx.reshape(B, C, 1), D, axis=2)
    x_sel = jnp.take_along_axis(x, idx_e, axis=1)
    g = _silu(x_sel @ w_gate)
    u = x_sel @ w_up
    y = (g * u) @ w_down
    r_sel = _sigmoid(jnp.take_along_axis(r, idx, axis=1))
    y = y * r_sel.reshape(B, C, 1)
    b_off = (jnp.arange(B) * S).reshape(B, 1)
    flat_idx = (idx + b_off).reshape(B * C)
    zero = (x * 0.0).reshape(B * S, D)
    upd = _scatter_add(zero, flat_idx, y.reshape(B * C, D), axis=0)
    return x + upd.reshape(B, S, D)
```

```python
import jax
import jax.numpy as jnp
from jax import lax
import jax.experimental.pallas as pl
import jax.experimental.pallas.tpu as pltpu

CAPACITY = 8
LANES = 128
INT_MIN = -(2**31)
F_CHUNK = 512
EARLY_ROWS = 384
LAST_ROWS = 32


def _kernel(x_hbm, wr_hbm, wg_hbm, wu_hbm, wd_hbm, o_hbm,
            x_v, wr_v, wg_v, wu_v, wd_v, xs_v, g_v, h_v, sems):
    D, S = x_v.shape
    F = wg_v.shape[1]
    n_bands = EARLY_ROWS // LANES
    tail = [(r, min(r + LANES, D)) for r in range(EARLY_ROWS, D, LANES)]
    cuts = sorted({r for r, _ in tail} | {D - LAST_ROWS, D})
    tail_rows = list(zip(cuts[:-1], cuts[1:]))

    cp_x = pltpu.make_async_copy(x_hbm, x_v, sems.at[0])
    cp_r = pltpu.make_async_copy(wr_hbm, wr_v, sems.at[1])
    cp_g = pltpu.make_async_copy(wg_hbm, wg_v, sems.at[2])
    cp_u = pltpu.make_async_copy(wu_hbm, wu_v, sems.at[3])

    def cp_band(i):
        r0 = i * LANES if isinstance(i, int) else pl.multiple_of(i * LANES, LANES)
        rows = pl.ds(r0, LANES)
        return pltpu.make_async_copy(wd_hbm.at[rows], wd_v.at[rows], sems.at[5 + i])

    cp_tail = [pltpu.make_async_copy(wd_hbm.at[a:b], wd_v.at[a:b], sems.at[5 + n_bands + i])
               for i, (a, b) in enumerate(tail_rows)]
    for cp in [cp_x, cp_r, cp_g, cp_u] + [cp_band(i) for i in range(n_bands)] + cp_tail:
        cp.start()

    cp_x.wait()
    cp_r.wait()

    sub = lax.broadcasted_iota(jnp.int32, (8, LANES), 0)
    lane = lax.broadcasted_iota(jnp.int32, (8, LANES), 1)

    w = jnp.broadcast_to(wr_v[...].astype(jnp.float32).reshape(1, D), (8, D)).astype(x_v.dtype)
    keys = []
    for v in range(S // (8 * LANES)):
        def score(jj, acc, v=v):
            c0 = pl.multiple_of(v * 8 * LANES + jj * 4 * LANES, 4 * LANES)
            r = jnp.dot(w, x_v[:, pl.ds(c0, 4 * LANES)], preferred_element_type=jnp.float32)
            for q in range(4):
                acc = jnp.where(sub == jj * 4 + q, r[:, q * LANES:(q + 1) * LANES], acc)
            return acc
        r = lax.fori_loop(0, 2, score, jnp.zeros((8, LANES), jnp.float32))
        r = r.astype(jnp.bfloat16).astype(jnp.float32)
        bits = pltpu.bitcast(r, jnp.int32)
        mono = jnp.where(bits < 0, INT_MIN - bits, bits)
        mono = jnp.where(r != r, INT_MIN + 65536, mono)
        keys.append(mono + (S - 1 - ((v * 8 + sub) * LANES + lane)))

    picked = jnp.zeros((8, LANES), jnp.int32)
    toks = []
    for c in range(CAPACITY):
        m = keys[0]
        for k in keys[1:]:
            m = jnp.maximum(m, k)
        top = jnp.max(m)
        keys = [jnp.where(k == top, INT_MIN, k) for k in keys]
        toks.append((S - 1) - (top & 0xFFFF))
        picked = jnp.where(sub == c, top, picked)
    mono = picked & jnp.int32(-65536)
    r_top = pltpu.bitcast(jnp.where(mono < 0, INT_MIN - mono, mono), jnp.float32)
    r_gate = jax.nn.sigmoid(r_top).astype(jnp.bfloat16).astype(jnp.float32)
    col0 = [pl.multiple_of(t & -LANES, LANES) for t in toks]
    lanes = [t & (LANES - 1) for t in toks]

    GR = 64
    lane_g = lax.broadcasted_iota(jnp.int32, (GR // 2, LANES), 1)

    def gather(i, carry):
        rows = pl.ds(pl.multiple_of(i * GR, GR), GR)
        acc = jnp.zeros((GR // 2, LANES), jnp.int32)
        for c in range(CAPACITY):
            strip = pltpu.bitcast(x_v[rows, pl.ds(col0[c], LANES)], jnp.int32)
            acc = jnp.where(lane_g == c, pltpu.roll(strip, (c - lanes[c]) & (LANES - 1), 1), acc)
        xs_v[rows, :] = pltpu.bitcast(acc, jnp.bfloat16).astype(jnp.float32)
        return carry
    lax.fori_loop(0, D // GR, gather, 0)
    pad = -D % LANES
    xs_t = jnp.concatenate([xs_v[...], jnp.zeros((pad, LANES), jnp.float32)], axis=0)
    x_sel = xs_t.T[0:CAPACITY, 0:D].astype(x_v.dtype)

    def residual(i, carry):
        rows = pl.ds(pl.multiple_of(i * 16, 16), 16)
        xv = x_v[rows, :].astype(jnp.float32)
        x_v[rows, :] = (xv + xv * 0.0).astype(x_v.dtype)
        return carry
    lax.fori_loop(0, D // 16, residual, 0)

    cp_g.wait()

    def gate(j, carry):
        cols = pl.ds(pl.multiple_of(j * F_CHUNK, F_CHUNK), F_CHUNK)
        g = jnp.dot(x_sel, wg_v[:, cols], preferred_element_type=jnp.float32)
        g = g.astype(jnp.bfloat16).astype(jnp.float32)
        g_v[:, cols] = g * jax.nn.sigmoid(g)
        return carry
    lax.fori_loop(0, F // F_CHUNK, gate, 0)

    cp_u.wait()

    def up(j, carry):
        cols = pl.ds(pl.multiple_of(j * F_CHUNK, F_CHUNK), F_CHUNK)
        u = jnp.dot(x_sel, wu_v[:, cols], preferred_element_type=jnp.float32)
        u = u.astype(jnp.bfloat16).astype(jnp.float32)
        h_v[:, cols] = g_v[:, cols] * u
        return carry
    lax.fori_loop(0, F // F_CHUNK, up, 0)

    def down(a, n):
        rows = pl.ds(a, n)
        y = lax.dot_general(h_v[...].astype(jnp.bfloat16), wd_v[rows, :], (((1,), (1,)), ((), ())),
                            preferred_element_type=jnp.float32)
        y = y.astype(jnp.bfloat16).astype(jnp.float32) * r_gate[:, 0:n]
        y = y.astype(jnp.bfloat16).astype(jnp.float32)
        if n < LANES:
            y = jnp.concatenate([y, jnp.zeros((8, LANES - n), jnp.float32)], axis=1)
        y_t = jnp.concatenate([y, jnp.zeros((LANES - 8, LANES), jnp.float32)], axis=0).T[0:n]
        xs = xs_v[rows, :]
        new = pltpu.bitcast((xs + (xs * 0.0 + y_t)).astype(jnp.bfloat16), jnp.int32)
        lane_n = lax.broadcasted_iota(jnp.int32, (n // 2, LANES), 1)
        for c in range(CAPACITY):
            moved = pltpu.roll(new, (lanes[c] - c) & (LANES - 1), 1)
            cols = pl.ds(col0[c], LANES)
            cur = pltpu.bitcast(x_v[rows, cols], jnp.int32)
            x_v[rows, cols] = pltpu.bitcast(jnp.where(lane_n == lanes[c], moved, cur), jnp.bfloat16)

    def band(i, carry):
        cp_band(i).wait()
        down(pl.multiple_of(i * LANES, LANES), LANES)
        return carry
    lax.fori_loop(0, n_bands, band, 0)

    pending = list(tail)
    writing = False
    for (a, b), cp in zip(tail_rows, cp_tail):
        cp.wait()
        if b == D - LAST_ROWS:
            pltpu.make_async_copy(x_v.at[0:EARLY_ROWS], o_hbm.at[0:EARLY_ROWS], sems.at[4]).start()
            writing = True
        while writing and pending and pending[0][1] <= b:
            lo, hi = pending.pop(0)
            down(lo, hi - lo)
    pltpu.make_async_copy(x_v.at[EARLY_ROWS:D], o_hbm.at[EARLY_ROWS:D], sems.at[4]).start()
    pltpu.make_async_copy(x_v, o_hbm, sems.at[4]).wait()


@jax.jit
def pallas_standalone__moe_arch_mod__prompt_kernel(
    x: jax.Array,
    w_r: jax.Array,
    w_gate: jax.Array,
    w_up: jax.Array,
    w_down: jax.Array,
):
    B, S, D = x.shape
    F = w_gate.shape[1]
    assert B == 1
    any_spec = pl.BlockSpec(memory_space=pl.ANY)
    out_t = pl.pallas_call(
        _kernel,
        in_specs=[any_spec] * 5,
        out_specs=any_spec,
        out_shape=jax.ShapeDtypeStruct((D, S), x.dtype),
        scratch_shapes=[
            pltpu.VMEM((D, S), x.dtype),
            pltpu.VMEM((D,), w_r.dtype),
            pltpu.VMEM((D, F), w_gate.dtype),
            pltpu.VMEM((D, F), w_up.dtype),
            pltpu.VMEM((D, F), w_down.dtype),
            pltpu.VMEM((D, LANES), jnp.float32),
            pltpu.VMEM((8, F), jnp.float32),
            pltpu.VMEM((8, F), jnp.float32),
            pltpu.SemaphoreType.DMA((5 + pl.cdiv(D, LANES) + 1,)),
        ],
        compiler_params=pltpu.CompilerParams(
            vmem_limit_bytes=64 << 20,
            disable_semaphore_checks=True,
        ),
    )(x.reshape(S, D).T, w_r, w_gate, w_up, w_down.T)
    return out_t.T.reshape(B, S, D)
```

```python
import jax
import jax.numpy as jnp
from jax import lax
import jax.experimental.pallas as pl
import jax.experimental.pallas.tpu as pltpu

CAPACITY = 8
LANES = 128
SUBLANES = 8
INT_MIN = -(2**31)
HIGH_HALF = -(2**16)

STREAMS = 4
BAND = LANES // STREAMS
EARLY_BANDS = 3
LAST_ROWS = 16
LAST_COLS = 3200
SIDE_COLS = 1792
WRITE_ROWS = 8
WRITE_COLS = 1024
F_CHUNK = 512
ROW_CHUNK = 16


def _round(v, dtype):
    return v.astype(dtype).astype(jnp.float32)


def _route(x_v, wr_v):
    ns, t, s = x_v.shape
    d = ns * t
    sub = lax.broadcasted_iota(jnp.int32, (SUBLANES, LANES), 0)
    lane = lax.broadcasted_iota(jnp.int32, (SUBLANES, LANES), 1)
    w = wr_v[...].astype(jnp.float32).reshape(1, d)
    w = jnp.broadcast_to(w, (SUBLANES, d)).astype(x_v.dtype)

    keys = []
    for v in range(s // (SUBLANES * LANES)):
        def score(j, acc, v=v):
            c0 = pl.multiple_of((v * SUBLANES + j * 4) * LANES, 4 * LANES)
            r = jnp.dot(w, x_v[:, :, pl.ds(c0, 4 * LANES)].reshape(d, 4 * LANES),
                        preferred_element_type=jnp.float32)
            for q in range(4):
                acc = jnp.where(sub == j * 4 + q, r[:, q * LANES:(q + 1) * LANES], acc)
            return acc

        r = lax.fori_loop(0, SUBLANES // 4, score, jnp.zeros((SUBLANES, LANES), jnp.float32))
        bits = pltpu.bitcast(_round(r, jnp.bfloat16), jnp.int32) & HIGH_HALF
        order = jnp.where(bits < 0, INT_MIN - bits, bits)
        order = jnp.where(r != r, INT_MIN - HIGH_HALF, order)
        keys.append(order + (s - 1 - ((v * SUBLANES + sub) * LANES + lane)))

    tokens = []
    picked = jnp.zeros((SUBLANES, LANES), jnp.int32)
    for c in range(CAPACITY):
        best = keys[0]
        for k in keys[1:]:
            best = jnp.maximum(best, k)
        top = jnp.max(best)
        keys = [jnp.where(k == top, INT_MIN, k) for k in keys]
        tokens.append((s - 1) - (top & ~HIGH_HALF))
        picked = jnp.where(sub == c, top, picked)
    order = picked & HIGH_HALF
    r_top = pltpu.bitcast(jnp.where(order < 0, INT_MIN - order, order), jnp.float32)
    return tokens, _round(jax.nn.sigmoid(r_top), x_v.dtype)


def _kernel(x_hbm, wr_hbm, wg_hbm, wu_hbm, wd_hbm, o_hbm,
            x_v, wr_v, wg_v, wu_v, wd_v, wd_s, xs_v, g_v, h_v, out_sem):
    ns, t, s = x_v.shape
    d = ns * t
    f = wg_v.shape[1]
    dtype = x_v.dtype
    early = EARLY_BANDS * BAND
    side = pl.ds(early - BAND, BAND)
    last = t - LAST_ROWS

    def write_rows(lo, hi):
        for r in range(lo, hi, WRITE_ROWS):
            for c in range(0, s, WRITE_COLS):
                piece = (slice(None), pl.ds(r, WRITE_ROWS), pl.ds(c, WRITE_COLS))
                pltpu.make_async_copy(x_v.at[piece], o_hbm.at[piece], out_sem).start()

    def body(sems, band_sems):
        def read_wd(rows, cols, sem):
            return pltpu.make_async_copy(wd_hbm.at[:, rows, cols], wd_v.at[:, rows, cols], sem)

        def band_rows(i):
            return pl.ds(i * BAND if isinstance(i, int) else pl.multiple_of(i * BAND, BAND), BAND)

        cp_x = pltpu.make_async_copy(x_hbm, x_v, sems.at[0])
        cp_wr = pltpu.make_async_copy(wr_hbm, wr_v, sems.at[1])
        cp_wg = pltpu.make_async_copy(wg_hbm, wg_v, sems.at[2])
        cp_wu = pltpu.make_async_copy(wu_hbm, wu_v, sems.at[3])
        cp_side_in = pltpu.make_async_copy(wd_hbm.at[:, side, pl.ds(0, SIDE_COLS)], wd_s, sems.at[4])
        cp_side_out = pltpu.make_async_copy(
            wd_s, wd_v.at[:, side, pl.ds(0, SIDE_COLS)], band_sems.at[EARLY_BANDS - 1])
        cp_late = read_wd(pl.ds(early, last - early), slice(None), sems.at[5])
        cp_last_a = read_wd(pl.ds(last, LAST_ROWS), pl.ds(0, f - LAST_COLS), sems.at[6])
        cp_last_b = read_wd(pl.ds(last, LAST_ROWS), pl.ds(f - LAST_COLS, LAST_COLS), sems.at[7])

        cp_x.start()
        cp_side_in.start()
        cp_wr.start()
        cp_wg.start()
        cp_wu.start()
        for i in range(EARLY_BANDS - 1):
            read_wd(band_rows(i), slice(None), band_sems.at[i]).start()
        read_wd(side, pl.ds(SIDE_COLS, f - SIDE_COLS), band_sems.at[EARLY_BANDS - 1]).start()
        cp_late.start()
        cp_last_a.start()
        cp_last_b.start()

        cp_x.wait()
        cp_wr.wait()
        tokens, r_gate = _route(x_v, wr_v)
        strips = [pl.multiple_of(tok & -LANES, LANES) for tok in tokens]
        lanes = [tok & (LANES - 1) for tok in tokens]

        def gather(i, carry):
            rows = pl.ds(pl.multiple_of(i * ROW_CHUNK, ROW_CHUNK), ROW_CHUNK)
            n = ns * ROW_CHUNK
            lane = lax.broadcasted_iota(jnp.int32, (n // 2, LANES), 1)
            acc = jnp.zeros((n // 2, LANES), jnp.int32)
            for c in range(CAPACITY):
                strip = x_v[:, rows, pl.ds(strips[c], LANES)].reshape(n, LANES)
                moved = pltpu.roll(pltpu.bitcast(strip, jnp.int32), (c - lanes[c]) & (LANES - 1), 1)
                acc = jnp.where(lane == c, moved, acc)
            xs_v[:, rows, :] = pltpu.bitcast(acc, dtype).astype(jnp.float32).reshape(ns, ROW_CHUNK, LANES)
            return carry

        lax.fori_loop(0, t // ROW_CHUNK, gather, 0)
        xs_t = jnp.concatenate(
            [xs_v[...].reshape(d, LANES), jnp.zeros((-d % LANES, LANES), jnp.float32)], axis=0)
        x_sel = xs_t.T[0:CAPACITY, 0:d].astype(dtype)

        def residual(i, carry):
            rows = pl.ds(pl.multiple_of(i * ROW_CHUNK, ROW_CHUNK), ROW_CHUNK)
            for k in range(ns):
                xv = x_v[k, rows, :].astype(jnp.float32)
                x_v[k, rows, :] = (xv + xv * 0.0).astype(dtype)
            return carry

        lax.fori_loop(0, t // ROW_CHUNK, residual, 0)

        cp_wg.wait()
        cp_side_in.wait()
        cp_side_out.start()

        def gate(j, carry):
            cols = pl.ds(pl.multiple_of(j * F_CHUNK, F_CHUNK), F_CHUNK)
            g = _round(jnp.dot(x_sel, wg_v[:, cols], preferred_element_type=jnp.float32), dtype)
            g_v[:, cols] = g * jax.nn.sigmoid(g)
            return carry

        lax.fori_loop(0, f // F_CHUNK, gate, 0)

        cp_wu.wait()

        def up(j, carry):
            cols = pl.ds(pl.multiple_of(j * F_CHUNK, F_CHUNK), F_CHUNK)
            u = _round(jnp.dot(x_sel, wu_v[:, cols], preferred_element_type=jnp.float32), dtype)
            h_v[:, cols] = g_v[:, cols] * u
            return carry

        lax.fori_loop(0, f // F_CHUNK, up, 0)

        def down(rows, m):
            n = ns * m
            y = lax.dot_general(h_v[...].astype(dtype), wd_v[:, rows, :].reshape(n, f),
                                (((1,), (1,)), ((), ())), preferred_element_type=jnp.float32)
            y = _round(_round(y, dtype) * r_gate[:, 0:n], dtype)
            if n < LANES:
                y = jnp.concatenate([y, jnp.zeros((CAPACITY, LANES - n), jnp.float32)], axis=1)
            y_t = jnp.concatenate([y, jnp.zeros((LANES - CAPACITY, LANES), jnp.float32)], axis=0).T[0:n]
            xs = xs_v[:, rows, :].reshape(n, LANES)
            new = pltpu.bitcast((xs + (xs * 0.0 + y_t)).astype(dtype), jnp.int32)
            lane = lax.broadcasted_iota(jnp.int32, (n // 2, LANES), 1)
            for c in range(CAPACITY):
                cols = pl.ds(strips[c], LANES)
                moved = pltpu.roll(new, (lanes[c] - c) & (LANES - 1), 1)
                cur = pltpu.bitcast(x_v[:, rows, cols].reshape(n, LANES), jnp.int32)
                out = pltpu.bitcast(jnp.where(lane == lanes[c], moved, cur), dtype)
                x_v[:, rows, cols] = out.reshape(ns, m, LANES)

        def band(i, carry):
            read_wd(band_rows(i), slice(None), band_sems.at[i]).wait()
            down(band_rows(i), BAND)
            return carry

        lax.fori_loop(0, EARLY_BANDS, band, 0)

        cp_late.wait()
        cp_last_a.wait()
        write_rows(0, early)
        down(pl.ds(early, last - early), last - early)
        cp_last_b.wait()
        down(pl.ds(last, LAST_ROWS), LAST_ROWS)
        write_rows(early, t)

    pl.run_scoped(body, pltpu.SemaphoreType.DMA((8,)), pltpu.SemaphoreType.DMA((EARLY_BANDS,)))
    pltpu.make_async_copy(x_v, o_hbm, out_sem).wait()


@jax.jit
def pallas_standalone__moe_arch_mod__prompt_kernel(
    x: jax.Array,
    w_r: jax.Array,
    w_gate: jax.Array,
    w_up: jax.Array,
    w_down: jax.Array,
):
    B, S, D = x.shape
    F = w_gate.shape[1]
    T = D // STREAMS
    assert B == 1 and x.dtype == jnp.bfloat16
    assert T == (EARLY_BANDS + 1) * BAND + LAST_ROWS
    any_spec = pl.BlockSpec(memory_space=pl.ANY)
    out_t = pl.pallas_call(
        _kernel,
        in_specs=[any_spec] * 5,
        out_specs=any_spec,
        out_shape=jax.ShapeDtypeStruct((STREAMS, T, S), x.dtype),
        scratch_shapes=[
            pltpu.VMEM((STREAMS, T, S), x.dtype),
            pltpu.VMEM((D,), w_r.dtype),
            pltpu.VMEM((D, F), w_gate.dtype),
            pltpu.VMEM((D, F), w_up.dtype),
            pltpu.VMEM((STREAMS, T, F), w_down.dtype),
            pltpu.SMEM((STREAMS, BAND, SIDE_COLS), w_down.dtype),
            pltpu.VMEM((STREAMS, T, LANES), jnp.float32),
            pltpu.VMEM((CAPACITY, F), jnp.float32),
            pltpu.VMEM((CAPACITY, F), jnp.float32),
            pltpu.SemaphoreType.DMA(()),
        ],
        compiler_params=pltpu.CompilerParams(vmem_limit_bytes=64 << 20),
    )(
        x.reshape(S, D).T.reshape(STREAMS, T, S),
        w_r,
        w_gate,
        w_up,
        w_down.T.reshape(STREAMS, T, F),
    )
    return out_t.reshape(D, S).T.reshape(B, S, D)
```

```python
import jax
import jax.numpy as jnp
from jax import lax
import jax.experimental.pallas as pl
import jax.experimental.pallas.tpu as pltpu

CAPACITY = 8
LANES = 128
SUBLANES = 8
INT_MIN = -(2**31)
HIGH_HALF = -(2**16)

STREAMS = 4
BAND = LANES // STREAMS
EARLY_BANDS = 3
LAST_ROWS = 16
LAST_COLS = 3200
SIDE_COLS = 1792
WRITE_ROWS = 8
WRITE_COLS = 1024
F_CHUNK = 512
ROW_CHUNK = 16


def _round(v, dtype):
    return v.astype(dtype).astype(jnp.float32)


def _route(x_v, wr_v):
    ns, t, s = x_v.shape
    d = ns * t
    sub = lax.broadcasted_iota(jnp.int32, (SUBLANES, LANES), 0)
    lane = lax.broadcasted_iota(jnp.int32, (SUBLANES, LANES), 1)
    w = wr_v[...].astype(jnp.float32).reshape(1, d)
    w = jnp.broadcast_to(w, (SUBLANES, d)).astype(x_v.dtype)

    keys = []
    for v in range(s // (SUBLANES * LANES)):
        def score(j, acc, v=v):
            c0 = pl.multiple_of((v * SUBLANES + j * 4) * LANES, 4 * LANES)
            r = jnp.dot(w, x_v[:, :, pl.ds(c0, 4 * LANES)].reshape(d, 4 * LANES),
                        preferred_element_type=jnp.float32)
            for q in range(4):
                acc = jnp.where(sub == j * 4 + q, r[:, q * LANES:(q + 1) * LANES], acc)
            return acc

        r = lax.fori_loop(0, SUBLANES // 4, score, jnp.zeros((SUBLANES, LANES), jnp.float32))
        bits = pltpu.bitcast(_round(r, jnp.bfloat16), jnp.int32) & HIGH_HALF
        order = jnp.where(bits < 0, INT_MIN - bits, bits)
        order = jnp.where(r != r, INT_MIN - HIGH_HALF, order)
        keys.append(order + (s - 1 - ((v * SUBLANES + sub) * LANES + lane)))

    tokens = []
    picked = jnp.zeros((SUBLANES, LANES), jnp.int32)
    for c in range(CAPACITY):
        best = keys[0]
        for k in keys[1:]:
            best = jnp.maximum(best, k)
        top = jnp.max(best)
        keys = [jnp.where(k == top, INT_MIN, k) for k in keys]
        tokens.append((s - 1) - (top & ~HIGH_HALF))
        picked = jnp.where(sub == c, top, picked)
    order = picked & HIGH_HALF
    r_top = pltpu.bitcast(jnp.where(order < 0, INT_MIN - order, order), jnp.float32)
    return tokens, _round(jax.nn.sigmoid(r_top), x_v.dtype)


def _kernel(x_hbm, wr_hbm, wg_hbm, wu_hbm, wd_hbm, o_hbm,
            x_v, wr_v, wg_v, wu_v, wd_v, wd_s, xs_v, g_v, h_v, out_sem):
    ns, t, s = x_v.shape
    d = ns * t
    f = wg_v.shape[1]
    dtype = x_v.dtype
    early = EARLY_BANDS * BAND
    side = pl.ds(early - BAND, BAND)
    last = t - LAST_ROWS

    def write_rows(lo, hi):
        for r in range(lo, hi, WRITE_ROWS):
            for c in range(0, s, WRITE_COLS):
                piece = (slice(None), pl.ds(r, WRITE_ROWS), pl.ds(c, WRITE_COLS))
                pltpu.make_async_copy(x_v.at[piece], o_hbm.at[piece], out_sem).start()

    def body(sems):
        def band_sem(i):
            return sems.at[8 + i]

        def read_wd(rows, cols, sem):
            return pltpu.make_async_copy(wd_hbm.at[:, rows, cols], wd_v.at[:, rows, cols], sem)

        def band_rows(i):
            return pl.ds(i * BAND if isinstance(i, int) else pl.multiple_of(i * BAND, BAND), BAND)

        cp_x = pltpu.make_async_copy(x_hbm, x_v, sems.at[0])
        cp_wr = pltpu.make_async_copy(wr_hbm, wr_v, sems.at[1])
        cp_wg = pltpu.make_async_copy(wg_hbm, wg_v, sems.at[2])
        cp_wu = pltpu.make_async_copy(wu_hbm, wu_v, sems.at[3])
        cp_side_in = pltpu.make_async_copy(wd_hbm.at[:, side, pl.ds(0, SIDE_COLS)], wd_s, sems.at[4])
        cp_side_out = pltpu.make_async_copy(
            wd_s, wd_v.at[:, side, pl.ds(0, SIDE_COLS)], band_sem(EARLY_BANDS - 1))
        cp_late = read_wd(pl.ds(early, last - early), slice(None), sems.at[5])
        cp_last_a = read_wd(pl.ds(last, LAST_ROWS), pl.ds(0, f - LAST_COLS), sems.at[6])
        cp_last_b = read_wd(pl.ds(last, LAST_ROWS), pl.ds(f - LAST_COLS, LAST_COLS), sems.at[7])

        cp_x.start()
        cp_side_in.start()
        cp_wr.start()
        cp_wg.start()
        cp_wu.start()
        for i in range(EARLY_BANDS - 1):
            read_wd(band_rows(i), slice(None), band_sem(i)).start()
        read_wd(side, pl.ds(SIDE_COLS, f - SIDE_COLS), band_sem(EARLY_BANDS - 1)).start()
        cp_late.start()
        cp_last_a.start()
        cp_last_b.start()

        cp_x.wait()
        cp_wr.wait()
        tokens, r_gate = _route(x_v, wr_v)
        strips = [pl.multiple_of(tok & -LANES, LANES) for tok in tokens]
        lanes = [tok & (LANES - 1) for tok in tokens]

        def gather(i, carry):
            rows = pl.ds(pl.multiple_of(i * ROW_CHUNK, ROW_CHUNK), ROW_CHUNK)
            n = ns * ROW_CHUNK
            lane = lax.broadcasted_iota(jnp.int32, (n // 2, LANES), 1)
            acc = jnp.zeros((n // 2, LANES), jnp.int32)
            for c in range(CAPACITY):
                strip = x_v[:, rows, pl.ds(strips[c], LANES)].reshape(n, LANES)
                moved = pltpu.roll(pltpu.bitcast(strip, jnp.int32), (c - lanes[c]) & (LANES - 1), 1)
                acc = jnp.where(lane == c, moved, acc)
            xs_v[:, rows, :] = pltpu.bitcast(acc, dtype).astype(jnp.float32).reshape(ns, ROW_CHUNK, LANES)
            return carry

        lax.fori_loop(0, t // ROW_CHUNK, gather, 0)
        xs_t = jnp.concatenate(
            [xs_v[...].reshape(d, LANES), jnp.zeros((-d % LANES, LANES), jnp.float32)], axis=0)
        x_sel = xs_t.T[0:CAPACITY, 0:d].astype(dtype)

        def residual(i, carry):
            rows = pl.ds(pl.multiple_of(i * ROW_CHUNK, ROW_CHUNK), ROW_CHUNK)
            for k in range(ns):
                xv = x_v[k, rows, :].astype(jnp.float32)
                x_v[k, rows, :] = (xv + xv * 0.0).astype(dtype)
            return carry

        lax.fori_loop(0, t // ROW_CHUNK, residual, 0)

        cp_wg.wait()
        cp_side_in.wait()
        cp_side_out.start()

        def gate(j, carry):
            cols = pl.ds(pl.multiple_of(j * F_CHUNK, F_CHUNK), F_CHUNK)
            g = _round(jnp.dot(x_sel, wg_v[:, cols], preferred_element_type=jnp.float32), dtype)
            g_v[:, cols] = g * jax.nn.sigmoid(g)
            return carry

        lax.fori_loop(0, f // F_CHUNK, gate, 0)

        cp_wu.wait()

        def up(j, carry):
            cols = pl.ds(pl.multiple_of(j * F_CHUNK, F_CHUNK), F_CHUNK)
            u = _round(jnp.dot(x_sel, wu_v[:, cols], preferred_element_type=jnp.float32), dtype)
            h_v[:, cols] = g_v[:, cols] * u
            return carry

        lax.fori_loop(0, f // F_CHUNK, up, 0)

        def down(rows, m):
            n = ns * m
            y = lax.dot_general(h_v[...].astype(dtype), wd_v[:, rows, :].reshape(n, f),
                                (((1,), (1,)), ((), ())), preferred_element_type=jnp.float32)
            y = _round(_round(y, dtype) * r_gate[:, 0:n], dtype)
            if n < LANES:
                y = jnp.concatenate([y, jnp.zeros((CAPACITY, LANES - n), jnp.float32)], axis=1)
            y_t = jnp.concatenate([y, jnp.zeros((LANES - CAPACITY, LANES), jnp.float32)], axis=0).T[0:n]
            xs = xs_v[:, rows, :].reshape(n, LANES)
            new = pltpu.bitcast((xs + (xs * 0.0 + y_t)).astype(dtype), jnp.int32)
            lane = lax.broadcasted_iota(jnp.int32, (n // 2, LANES), 1)
            for c in range(CAPACITY):
                cols = pl.ds(strips[c], LANES)
                moved = pltpu.roll(new, (lanes[c] - c) & (LANES - 1), 1)
                cur = pltpu.bitcast(x_v[:, rows, cols].reshape(n, LANES), jnp.int32)
                out = pltpu.bitcast(jnp.where(lane == lanes[c], moved, cur), dtype)
                x_v[:, rows, cols] = out.reshape(ns, m, LANES)

        def band(i, carry):
            read_wd(band_rows(i), slice(None), band_sem(i)).wait()
            down(band_rows(i), BAND)
            return carry

        lax.fori_loop(0, EARLY_BANDS, band, 0)

        cp_late.wait()
        cp_last_a.wait()
        write_rows(0, early)
        down(pl.ds(early, last - early), last - early)
        cp_last_b.wait()
        down(pl.ds(last, LAST_ROWS), LAST_ROWS)
        write_rows(early, t)

    pl.run_scoped(body, pltpu.SemaphoreType.DMA((8 + EARLY_BANDS,)))
    pltpu.make_async_copy(x_v, o_hbm, out_sem).wait()


@jax.jit
def pallas_standalone__moe_arch_mod__prompt_kernel(
    x: jax.Array,
    w_r: jax.Array,
    w_gate: jax.Array,
    w_up: jax.Array,
    w_down: jax.Array,
):
    B, S, D = x.shape
    F = w_gate.shape[1]
    T = D // STREAMS
    assert B == 1 and x.dtype == jnp.bfloat16
    assert T == (EARLY_BANDS + 1) * BAND + LAST_ROWS
    any_spec = pl.BlockSpec(memory_space=pl.ANY)
    out_t = pl.pallas_call(
        _kernel,
        in_specs=[any_spec] * 5,
        out_specs=any_spec,
        out_shape=jax.ShapeDtypeStruct((STREAMS, T, S), x.dtype),
        scratch_shapes=[
            pltpu.VMEM((STREAMS, T, S), x.dtype),
            pltpu.VMEM((D,), w_r.dtype),
            pltpu.VMEM((D, F), w_gate.dtype),
            pltpu.VMEM((D, F), w_up.dtype),
            pltpu.VMEM((STREAMS, T, F), w_down.dtype),
            pltpu.SMEM((STREAMS, BAND, SIDE_COLS), w_down.dtype),
            pltpu.VMEM((STREAMS, T, LANES), jnp.float32),
            pltpu.VMEM((CAPACITY, F), jnp.float32),
            pltpu.VMEM((CAPACITY, F), jnp.float32),
            pltpu.SemaphoreType.DMA(()),
        ],
        compiler_params=pltpu.CompilerParams(vmem_limit_bytes=64 << 20),
    )(
        x.reshape(S, D).T.reshape(STREAMS, T, S),
        w_r,
        w_gate,
        w_up,
        w_down.T.reshape(STREAMS, T, F),
    )
    return out_t.reshape(D, S).T.reshape(B, S, D)
```

```python
import jax
import jax.numpy as jnp
from jax import lax
import jax.experimental.pallas as pl
import jax.experimental.pallas.tpu as pltpu

CAPACITY = 8
LANES = 128
SUBLANES = 8
INT_MIN = -(2**31)
HIGH_HALF = -(2**16)

STREAMS = 4
BAND = LANES // STREAMS
EARLY_BANDS = 2
COPY_ROWS = 8
FFN_STREAMS = 6
FFN_COLS = 1536
READ_COLS = 2304
WRITE_COLS = 1024
LAST_COLS = 768
F_CHUNK = 512
ROW_CHUNK = 16


def _round(v, dtype):
    return v.astype(dtype).astype(jnp.float32)


def _route(x_v, wr_v):
    ns, t, s = x_v.shape
    d = ns * t
    sub = lax.broadcasted_iota(jnp.int32, (SUBLANES, LANES), 0)
    lane = lax.broadcasted_iota(jnp.int32, (SUBLANES, LANES), 1)
    w = wr_v[...].astype(jnp.float32).reshape(1, d)
    w = jnp.broadcast_to(w, (SUBLANES, d)).astype(x_v.dtype)

    keys = []
    for v in range(s // (SUBLANES * LANES)):
        def score(j, acc, v=v):
            c0 = pl.multiple_of((v * SUBLANES + j * 4) * LANES, 4 * LANES)
            r = jnp.dot(w, x_v[:, :, pl.ds(c0, 4 * LANES)].reshape(d, 4 * LANES),
                        preferred_element_type=jnp.float32)
            for q in range(4):
                acc = jnp.where(sub == j * 4 + q, r[:, q * LANES:(q + 1) * LANES], acc)
            return acc

        r = lax.fori_loop(0, SUBLANES // 4, score, jnp.zeros((SUBLANES, LANES), jnp.float32))
        bits = pltpu.bitcast(_round(r, jnp.bfloat16), jnp.int32) & HIGH_HALF
        order = jnp.where(bits < 0, INT_MIN - bits, bits)
        order = jnp.where(r != r, INT_MIN - HIGH_HALF, order)
        keys.append(order + (s - 1 - ((v * SUBLANES + sub) * LANES + lane)))

    tokens = []
    picked = jnp.zeros((SUBLANES, LANES), jnp.int32)
    for c in range(CAPACITY):
        best = keys[0]
        for k in keys[1:]:
            best = jnp.maximum(best, k)
        top = jnp.max(best)
        keys = [jnp.where(k == top, INT_MIN, k) for k in keys]
        tokens.append((s - 1) - (top & ~HIGH_HALF))
        picked = jnp.where(sub == c, top, picked)
    order = picked & HIGH_HALF
    r_top = pltpu.bitcast(jnp.where(order < 0, INT_MIN - order, order), jnp.float32)
    return tokens, _round(jax.nn.sigmoid(r_top), x_v.dtype)


def _kernel(x_hbm, wr_hbm, wg_hbm, wu_hbm, wd_hbm, o_hbm,
            x_v, wr_v, wg_v, wu_v, wd_v, wd_s, xs_v, g_v, h_v, out_sem):
    ns, t, s = x_v.shape
    d = ns * t
    _, t_ffn, f = wg_v.shape
    dtype = x_v.dtype
    n_bands = t // BAND
    late = (n_bands - 1) * BAND
    side = pl.ds(n_bands * BAND, t - n_bands * BAND)

    def copy(src, dst, sem, rows=slice(None), cols=slice(None)):
        return pltpu.make_async_copy(src.at[:, rows, cols], dst.at[:, rows, cols], sem)

    def start_rows(src, dst, sem, lo, hi, width):
        assert lo % COPY_ROWS == 0 and hi % COPY_ROWS == 0 and src.shape[2] % width == 0

        def step(i, carry):
            rows = pl.ds(pl.multiple_of(i * COPY_ROWS, COPY_ROWS), COPY_ROWS)
            for c in range(0, src.shape[2], width):
                copy(src, dst, sem, rows, pl.ds(c, width)).start()
            return carry

        lax.fori_loop(lo // COPY_ROWS, hi // COPY_ROWS, step, 0)

    def body(sems):
        (x_sem, wr_sem, wg_sem, wu_sem, side_in_sem, side_out_sem,
         late_sem, early_cut_sem, late_cut_sem, last_sem) = (sems.at[i] for i in range(10))

        def band_sem(i):
            return sems.at[10 + i]

        cp_wr = pltpu.make_async_copy(wr_hbm, wr_v, wr_sem)
        cp_side_in = pltpu.make_async_copy(wd_hbm.at[:, side], wd_s, side_in_sem)
        cp_side_out = pltpu.make_async_copy(wd_s, wd_v.at[:, side], side_out_sem)

        copy(x_hbm, x_v, x_sem, pl.ds(0, COPY_ROWS)).start()
        cp_side_in.start()
        cp_wr.start()
        start_rows(x_hbm, x_v, x_sem, COPY_ROWS, t, s)
        start_rows(wg_hbm, wg_v, wg_sem, 0, t_ffn, FFN_COLS)

        copy(x_hbm, x_v, x_sem).wait()
        cp_wr.wait()
        tokens, r_gate = _route(x_v, wr_v)
        strips = [pl.multiple_of(jnp.clip(tok & -LANES, 0, s - LANES), LANES) for tok in tokens]
        lanes = [tok & (LANES - 1) for tok in tokens]

        def gather(i, carry):
            rows = pl.ds(pl.multiple_of(i * ROW_CHUNK, ROW_CHUNK), ROW_CHUNK)
            n = ns * ROW_CHUNK
            lane = lax.broadcasted_iota(jnp.int32, (n // 2, LANES), 1)
            acc = jnp.zeros((n // 2, LANES), jnp.int32)
            for c in range(CAPACITY):
                strip = x_v[:, rows, pl.ds(strips[c], LANES)].reshape(n, LANES)
                moved = pltpu.roll(pltpu.bitcast(strip, jnp.int32), (c - lanes[c]) & (LANES - 1), 1)
                acc = jnp.where(lane == c, moved, acc)
            xs_v[:, rows, :] = pltpu.bitcast(acc, dtype).astype(jnp.float32).reshape(ns, ROW_CHUNK, LANES)
            return carry

        lax.fori_loop(0, t // ROW_CHUNK, gather, 0)
        xs_t = jnp.concatenate(
            [xs_v[...].reshape(d, LANES), jnp.zeros((-d % LANES, LANES), jnp.float32)], axis=0)
        x_sel = xs_t.T[0:CAPACITY, 0:d].astype(dtype)

        def residual(i, carry):
            rows = pl.ds(pl.multiple_of(i * ROW_CHUNK, ROW_CHUNK), ROW_CHUNK)
            for k in range(ns):
                xv = x_v[k, rows, :].astype(jnp.float32)
                x_v[k, rows, :] = (xv + xv * 0.0).astype(dtype)
            return carry

        lax.fori_loop(0, t // ROW_CHUNK, residual, 0)

        start_rows(wu_hbm, wu_v, wu_sem, 0, 2 * t_ffn // 3, FFN_COLS)
        copy(wg_hbm, wg_v, wg_sem).wait()
        cp_side_in.wait()
        cp_side_out.start()
        start_rows(wu_hbm, wu_v, wu_sem, 2 * t_ffn // 3, t_ffn, FFN_COLS)

        def gate(j, carry):
            cols = pl.ds(pl.multiple_of(j * F_CHUNK, F_CHUNK), F_CHUNK)
            g = _round(jnp.dot(x_sel, wg_v[:, :, cols].reshape(d, F_CHUNK),
                               preferred_element_type=jnp.float32), dtype)
            g_v[:, cols] = g * jax.nn.sigmoid(g)
            return carry

        lax.fori_loop(0, f // F_CHUNK, gate, 0)

        for i in range(n_bands - 1):
            start_rows(wd_hbm, wd_v, band_sem(i), i * BAND, (i + 1) * BAND, READ_COLS)
        last = late + BAND - COPY_ROWS
        prev = pl.ds(last - COPY_ROWS, COPY_ROWS)
        cp_early_cut = copy(wd_hbm, wd_v, early_cut_sem, prev, pl.ds(0, f - LAST_COLS))
        cp_late_cut = copy(wd_hbm, wd_v, late_cut_sem, prev, pl.ds(f - LAST_COLS, LAST_COLS))
        start_rows(wd_hbm, wd_v, late_sem, late, last - COPY_ROWS, READ_COLS)
        cp_early_cut.start()
        cp_late_cut.start()
        start_rows(wd_hbm, wd_v, last_sem, last, last + COPY_ROWS, READ_COLS)

        copy(wu_hbm, wu_v, wu_sem).wait()

        def up(j, carry):
            cols = pl.ds(pl.multiple_of(j * F_CHUNK, F_CHUNK), F_CHUNK)
            u = _round(jnp.dot(x_sel, wu_v[:, :, cols].reshape(d, F_CHUNK),
                               preferred_element_type=jnp.float32), dtype)
            h_v[:, cols] = g_v[:, cols] * u
            return carry

        lax.fori_loop(0, f // F_CHUNK, up, 0)

        def down(rows, m):
            n = ns * m
            y = lax.dot_general(h_v[...].astype(dtype), wd_v[:, rows, :].reshape(n, f),
                                (((1,), (1,)), ((), ())), preferred_element_type=jnp.float32)
            y = _round(_round(y, dtype) * r_gate[:, 0:n], dtype)
            if n < LANES:
                y = jnp.concatenate([y, jnp.zeros((CAPACITY, LANES - n), jnp.float32)], axis=1)
            y_t = jnp.concatenate([y, jnp.zeros((LANES - CAPACITY, LANES), jnp.float32)], axis=0).T[0:n]
            xs = xs_v[:, rows, :].reshape(n, LANES)
            new = pltpu.bitcast((xs + (xs * 0.0 + y_t)).astype(dtype), jnp.int32)
            lane = lax.broadcasted_iota(jnp.int32, (n // 2, LANES), 1)
            for c in range(CAPACITY):
                cols = pl.ds(strips[c], LANES)
                moved = pltpu.roll(new, (lanes[c] - c) & (LANES - 1), 1)
                cur = pltpu.bitcast(x_v[:, rows, cols].reshape(n, LANES), jnp.int32)
                out = pltpu.bitcast(jnp.where(lane == lanes[c], moved, cur), dtype)
                x_v[:, rows, cols] = out.reshape(ns, m, LANES)

        def band(i, carry):
            @pl.when(i == EARLY_BANDS)
            def _():
                cp_early_cut.wait()
                start_rows(x_v, o_hbm, out_sem, 0, EARLY_BANDS * BAND, WRITE_COLS)

            rows = pl.ds(pl.multiple_of(i * BAND, BAND), BAND)
            copy(wd_hbm, wd_v, band_sem(i), rows).wait()
            down(rows, BAND)
            return carry

        lax.fori_loop(0, n_bands - 1, band, 0)
        start_rows(x_v, o_hbm, out_sem, EARLY_BANDS * BAND, late, WRITE_COLS)

        copy(wd_hbm, wd_v, late_sem, pl.ds(late, last - COPY_ROWS - late)).wait()
        cp_late_cut.wait()
        copy(wd_hbm, wd_v, last_sem, pl.ds(last, COPY_ROWS)).wait()
        down(pl.ds(late, BAND), BAND)
        start_rows(x_v, o_hbm, out_sem, late, late + BAND, WRITE_COLS)

        cp_side_out.wait()
        down(side, side.size)
        start_rows(x_v, o_hbm, out_sem, late + BAND, t, WRITE_COLS)

    pl.run_scoped(body, pltpu.SemaphoreType.DMA((10 + n_bands - 1,)))
    pltpu.make_async_copy(x_v, o_hbm, out_sem).wait()


@jax.jit
def pallas_standalone__moe_arch_mod__prompt_kernel(
    x: jax.Array,
    w_r: jax.Array,
    w_gate: jax.Array,
    w_up: jax.Array,
    w_down: jax.Array,
):
    B, S, D = x.shape
    F = w_gate.shape[1]
    T = D // STREAMS
    ffn_shape = (FFN_STREAMS, D // FFN_STREAMS, F)
    assert B == 1 and x.dtype == jnp.bfloat16
    assert T % BAND and EARLY_BANDS < T // BAND - 1
    any_spec = pl.BlockSpec(memory_space=pl.ANY)
    out_t = pl.pallas_call(
        _kernel,
        in_specs=[any_spec] * 5,
        out_specs=any_spec,
        out_shape=jax.ShapeDtypeStruct((STREAMS, T, S), x.dtype),
        scratch_shapes=[
            pltpu.VMEM((STREAMS, T, S), x.dtype),
            pltpu.VMEM((D,), w_r.dtype),
            pltpu.VMEM(ffn_shape, w_gate.dtype),
            pltpu.VMEM(ffn_shape, w_up.dtype),
            pltpu.VMEM((STREAMS, T, F), w_down.dtype),
            pltpu.SMEM((STREAMS, T % BAND, F), w_down.dtype),
            pltpu.VMEM((STREAMS, T, LANES), jnp.float32),
            pltpu.VMEM((CAPACITY, F), jnp.float32),
            pltpu.VMEM((CAPACITY, F), jnp.float32),
            pltpu.SemaphoreType.DMA(()),
        ],
        compiler_params=pltpu.CompilerParams(vmem_limit_bytes=64 << 20),
    )(
        x.reshape(S, D).T.reshape(STREAMS, T, S),
        w_r,
        w_gate.reshape(ffn_shape),
        w_up.reshape(ffn_shape),
        w_down.T.reshape(STREAMS, T, F),
    )
    return out_t.reshape(D, S).T.reshape(B, S, D)
```
